```python
import os as _os
_os.environ.setdefault("JAX_PLATFORMS", "cpu")
import jax
import jax.numpy as jnp

def _softmax(x, axis=-1):
    return jax.nn.softmax(x, axis=axis)
def _gelu(x):
    return jax.nn.gelu(x, approximate=True)
def _silu(x):
    return jax.nn.silu(x)
def _sigmoid(x):
    return jax.nn.sigmoid(x)
def _layernorm(x, axis=-1, eps=1e-5):
    m = jnp.mean(x, axis=axis, keepdims=True)
    v = jnp.var(x, axis=axis, keepdims=True)
    return (x - m) / jnp.sqrt(v + eps)
def _scatter_add(tgt, idx, src, axis=0):
    return tgt.at[idx].add(src)
def _segment_sum(src, seg, n):
    return jax.ops.segment_sum(src, seg, n)
class _Rng:
    def __init__(self, key):
        self._k = key
    def _next(self):
        self._k, sub = jax.random.split(self._k)
        return sub
    def normal(self, shape):
        return jax.random.normal(self._next(), shape, dtype=jnp.bfloat16)
    def randint(self, lo, hi, shape):
        return jax.random.randint(self._next(), shape, lo, hi, dtype=jnp.int32)
    def uniform(self, shape, lo=0.0, hi=1.0):
        return jax.random.uniform(self._next(), shape, jnp.bfloat16, lo, hi)
    def permutation(self, n):
        return jax.random.permutation(self._next(), n)


kernel_name = 'concat_heads__spectral_gfnet__sliding_block__prompt'

def setup_inputs():
    _rng = _Rng(jax.random.key(int.from_bytes(__import__("os").urandom(4), "little")))
    _w = (lambda a: (lambda t: t.astype(jnp.bfloat16) if jnp.issubdtype(t.dtype, jnp.floating) else t)(jnp.asarray(a)))
    def _A_setup():
        B, S, D = 1, 2048, 640
        Df = D // 2 + 1
        return {
            "x": _w((lambda *s: _rng.normal(s) * 0.05)(B, S, D)),
            "w_r": _w((lambda *s: _rng.normal(s) * 0.4)(S, Df) * 0.02),
            "w_i": _w((lambda *s: _rng.normal(s) * 0.4)(S, Df) * 0.02),
        }
    _A_in = _A_setup()

    def _B_setup():
        B, S, D = 1, 2048, 640
        return {
            "x": _w((lambda *s: _rng.normal(s) * 0.2)(B, S, D)),
            "wqkv": _w((lambda *s: _rng.normal(s) * 0.2)(D, 3 * D)),
            "wo": _w((lambda *s: _rng.normal(s) * 0.05)(D, D)),
        }
    _B_in = _B_setup()

    return {
        "A_x": _A_in["x"],
        "A_w_r": _A_in["w_r"],
        "A_w_i": _A_in["w_i"],
        "B_x": _B_in["x"],
        "B_wqkv": _B_in["wqkv"],
        "B_wo": _B_in["wo"],
    }

def reference(A_x, A_w_r, A_w_i, B_x, B_wqkv, B_wo):
    def _A_ref(x, w_r, w_i):
        B, S, D = x.shape
        X = (lambda x, axes=(-2,-1): jnp.fft.rfft2(x.astype(jnp.float32), axes=axes))(x, axes=(-2, -1))
        W = w_r + 1j * w_i
        X = X * W
        y = (lambda x, s, axes=(-2,-1): jnp.fft.irfft2(x, s=s, axes=axes).astype(jnp.bfloat16))(X, (S, D), axes=(-2, -1))
        return y

    def _B_ref(x, wqkv, wo):
        B, S, D = x.shape
        H = 32; Dh = D // H; W = 256
        qkv = (lambda x, *d: x.transpose(*d))((x @ wqkv).reshape(B, S, 3, H, Dh), 2, 0, 3, 1, 4)
        q, k, v = qkv[0], qkv[1], qkv[2]
        scores = jnp.einsum("bhqd,bhkd->bhqk", q, k) * (Dh ** -0.5)
        idx = jnp.arange(S)
        mask = (idx[:, None] - idx[None, :] >= 0) & (idx[:, None] - idx[None, :] < W)
        scores = jnp.where(mask[None, None], scores, -1e9)
        p = _softmax(scores, axis=-1)
        o = jnp.einsum("bhqk,bhkd->bhqd", p, v)
        return (lambda x, *d: x.transpose(*d))(o, 0, 2, 1, 3).reshape(B, S, D) @ wo

    a = _A_ref(A_x, A_w_r, A_w_i)
    b = _B_ref(B_x, B_wqkv, B_wo)
    return jnp.concatenate([a, b], axis=-1)
```

```python
import numpy as np
import jax
import jax.numpy as jnp
from jax import lax
import jax.experimental.pallas as pl
import jax.experimental.pallas.tpu as pltpu

S = 2048
D = 640
DF = D // 2 + 1
PF = 384
H = 32
DH = 20
WIN = 256
N1 = 16
N2 = 128
G = 8
GR = 4 * DH
QB = 32
KW = WIN + QB
SP = S + WIN
NEG = -1e9
NXC = 4
R0 = 72
KR = 256 + R0
WR = 5 * R0
NOC = 4
VR = 80


def _constants():
    th = 2.0 * np.pi / D
    rows14 = np.concatenate([1 + 5 * np.arange(64), 4 + 5 * np.arange(64)])
    rows23 = np.concatenate([2 + 5 * np.arange(64), 3 + 5 * np.arange(64)])
    rows0 = 5 * np.arange(R0)
    ok0 = (rows0 <= D // 2).astype(np.float64)
    d2 = np.arange(128)
    sg = np.concatenate([np.ones(64), -np.ones(64)])

    def fwd_pair(rows):
        a = th * ((rows[:, None] * d2[None, :]) % D)
        c, sn = np.cos(a), np.sin(a)
        m = np.zeros((256, 256))
        m[:128, :128] = c
        m[:128, 128:] = sg[:, None] * sn
        m[128:, :128] = -sn
        m[128:, 128:] = sg[:, None] * c
        return m

    def inv_pair(rows):
        a = th * ((rows[:, None] * d2[None, :]) % D)
        c, sn = 2.0 * np.cos(a), 2.0 * np.sin(a)
        m = np.zeros((256, 256))
        m[:128, :128] = c
        m[128:, :128] = -sn
        m[:128, 128:] = sg[:, None] * sn
        m[128:, 128:] = sg[:, None] * c
        return m / (S * D)

    fp = np.stack([fwd_pair(rows14), fwd_pair(rows23)])
    gp = np.stack([inv_pair(rows14), inv_pair(rows23)])
    a0 = th * ((rows0[:, None] * d2[None, :]) % D)
    f0 = np.concatenate([np.cos(a0), -np.sin(a0)]) * np.tile(ok0, 2)[:, None]
    c0 = 2.0 * ok0.copy()
    c0[0] = 1.0
    c0[D // 2 // 5] = 1.0
    s0 = c0.copy()
    s0[0] = 0.0
    s0[D // 2 // 5] = 0.0
    g0 = np.zeros((256, 128))
    g0[:R0] = c0[:, None] * np.cos(a0)
    g0[128:128 + R0] = -s0[:, None] * np.sin(a0)
    g0 = g0 / (S * D)
    s1 = np.arange(N2)[:, None]
    k1 = np.arange(N2)[None, :]
    rf = np.zeros((N1, N2, 2 * N2))
    li = np.zeros((N1, 2 * N2, N2))
    for b in range(N1):
        a = 2.0 * np.pi * (((N1 * s1 + b) * k1) % S) / S
        rf[b, :, :N2] = np.cos(a)
        rf[b, :, N2:] = np.sin(a)
        li[b, :N2] = np.cos(a)
        li[b, N2:] = np.sin(a)
    pm = np.zeros((2, 128, 128))
    for b in range(N1):
        for l in range(8):
            pm[0, b * 8 + l, l * 16 + b] = 1.0
    pm[1] = pm[0].T
    hrow = (np.arange(GR) // DH)[:, None]
    slot = (np.arange(128) // QB)[None, :]
    mk = np.stack([(slot == (hrow + j) % 4) for j in range(4)]).astype(np.float32)
    bf = jnp.bfloat16
    return (jnp.asarray(fp, bf), jnp.asarray(f0, bf), jnp.asarray(gp, bf),
            jnp.asarray(g0, bf), jnp.asarray(rf, bf), jnp.asarray(li, bf),
            jnp.asarray(mk), jnp.asarray(pm, bf))


def _cmul_const(re, im, k, n, sign):
    k = k % n
    if k == 0:
        return re, im
    if 4 * k == n:
        return (-im, re) if sign > 0 else (im, -re)
    if 2 * k == n:
        return -re, -im
    if 4 * k == 3 * n:
        return (im, -re) if sign > 0 else (-im, re)
    c = float(np.cos(2 * np.pi * k / n))
    s = float(np.sin(2 * np.pi * k / n)) * sign
    if abs(abs(c) - abs(s)) < 1e-12:
        if s * c > 0:
            return (re - im) * c, (re + im) * c
        return (re + im) * c, (im - re) * c
    return re * c - im * s, re * s + im * c


def _fft_list(xs, sign):
    n = len(xs)
    if n == 1:
        return xs
    ev = _fft_list(xs[0::2], sign)
    od = _fft_list(xs[1::2], sign)
    out = [None] * n
    for k in range(n // 2):
        tr, ti = _cmul_const(od[k][0], od[k][1], k, n, sign)
        out[k] = (ev[k][0] + tr, ev[k][1] + ti)
        out[k + n // 2] = (ev[k][0] - tr, ev[k][1] - ti)
    return out


def _kernel(ax_hbm, wr_hbm, wi_hbm, bx_hbm, wqkv_hbm, wo_hbm,
            fp_hbm, f0_hbm, gp_hbm, g0_hbm, rf_hbm, li_hbm, mk_hbm, pm_hbm,
            out_hbm,
            ax_ref, wr_ref, wi_ref, bx_ref, wqkv_ref, wo_ref,
            fp_ref, f0_ref, gp_ref, g0_ref, rf_ref, li_ref, mk_ref, pm_ref,
            oa_ref, ob_ref, in_sems, out_sems, x_sems,
            x32_ref, tt_ref, xt_ref, a_ref, w32_ref, u_ref,
            qm_ref, vt_ref, kg_ref, ot_ref, sc0_ref, sc1_ref):
    f32 = jnp.float32
    bf = jnp.bfloat16

    XC = S // NXC

    def x_copy(c):
        return pltpu.make_async_copy(ax_hbm.at[pl.ds(c * XC, XC), :],
                                     ax_ref.at[pl.ds(c * XC, XC), :],
                                     x_sems.at[c])

    srcs = (pm_hbm, fp_hbm, f0_hbm, rf_hbm, wr_hbm, wi_hbm, li_hbm, gp_hbm,
            g0_hbm, bx_hbm, wqkv_hbm, mk_hbm, wo_hbm)
    dsts = (pm_ref, fp_ref, f0_ref, rf_ref, wr_ref, wi_ref, li_ref, gp_ref,
            g0_ref, bx_ref, wqkv_ref, mk_ref, wo_ref)
    cps = [pltpu.make_async_copy(s_, d_, in_sems.at[i])
           for i, (s_, d_) in enumerate(zip(srcs, dsts))]
    cps[0].start()
    for c in range(NXC):
        x_copy(c).start()

    c51 = float(np.cos(2 * np.pi / 5))
    c52 = float(np.cos(4 * np.pi / 5))
    s51 = float(np.sin(2 * np.pi / 5))
    s52 = float(np.sin(4 * np.pi / 5))
    nt = (((1,), (1,)), ((), ()))

    cps[0].wait()

    def rad5(m, carry):
        r0 = pl.multiple_of(m * 128, 128)
        xp = jnp.dot(pm_ref[0], ax_ref[pl.ds(r0, 128), :],
                     preferred_element_type=f32)
        xs = [xp[:, c * 128:(c + 1) * 128] for c in range(5)]
        a1 = xs[1] + xs[4]
        b1 = xs[1] - xs[4]
        a2 = xs[2] + xs[3]
        b2 = xs[2] - xs[3]
        ts = jnp.concatenate(
            (xs[0] + a1 + a2,
             xs[0] + c51 * a1 + c52 * a2,
             -(s51 * b1 + s52 * b2),
             xs[0] + c52 * a1 + c51 * a2,
             s51 * b2 - s52 * b1), axis=1)
        o0 = pl.multiple_of(m * 8, 8)
        for b in range(N1):
            tt_ref[pl.ds(b * N2 + o0, 8), :] = ts[b * 8:(b + 1) * 8]
        return carry

    for c in range(NXC):
        x_copy(c).wait()
        if c == NXC - 1:
            for c_ in cps[1:9]:
                c_.start()
        lax.fori_loop(c * (N1 // NXC), (c + 1) * (N1 // NXC), rad5, 0)
    for c_ in cps[9:]:
        c_.start()

    cps[1].wait()
    cps[2].wait()
    for p_ in range(2):
        xp = lax.dot_general(
            fp_ref[p_], tt_ref[:, pl.ds(128 + 256 * p_, 256)].astype(bf),
            nt, preferred_element_type=f32)
        xt_ref[pl.ds(128 * p_, 128), :] = xp[:128].astype(bf)
        xt_ref[pl.ds(KR + 128 * p_, 128), :] = xp[128:].astype(bf)
    x0 = lax.dot_general(f0_ref[...], tt_ref[:, pl.ds(0, 128)].astype(bf), nt,
                         preferred_element_type=f32)
    xt_ref[pl.ds(256, R0), :] = x0[:R0].astype(bf)
    xt_ref[pl.ds(KR + 256, R0), :] = x0[R0:].astype(bf)

    cps[3].wait()

    def sfwd(b, carry):
        c0 = pl.multiple_of(b * N2, N2)
        pq = jnp.dot(xt_ref[:, pl.ds(c0, N2)], rf_ref[b],
                     preferred_element_type=f32)
        a_ref[0, :, pl.ds(c0, N2)] = pq[:KR, :N2] + pq[KR:, N2:]
        a_ref[1, :, pl.ds(c0, N2)] = pq[KR:, :N2] - pq[:KR, N2:]
        return carry

    lax.fori_loop(0, N1, sfwd, 0)

    cps[4].wait()
    cps[5].wait()
    for p_, w_ref in enumerate((wr_ref, wi_ref)):
        for b in range(N1):
            w32_ref[p_, b, pl.ds(0, DF), :] = (
                w_ref[:, pl.ds(b * N2, N2)].astype(f32))
            w32_ref[p_, b, pl.ds(DF, WR - DF), :] = jnp.zeros((WR - DF, N2), f32)

    def filt(i, carry):
        r0 = pl.multiple_of(i * 8, 8)
        grp = i // 8
        k1 = jnp.where(grp == 0, 1, jnp.where(grp == 1, 4, jnp.where(
            grp == 2, 2, jnp.where(grp == 3, 3, 0))))
        jj = jnp.where(grp >= 4, r0 - 256, r0 - grp * 64)
        k0 = k1 + 5 * jj
        xs = [(a_ref[0, pl.ds(r0, 8), pl.ds(b * N2, N2)],
               a_ref[1, pl.ds(r0, 8), pl.ds(b * N2, N2)]) for b in range(N1)]
        ys = _fft_list(xs, -1)
        zs = []
        for b in range(N1):
            wr = w32_ref[0, b, pl.ds(k0, 8, stride=5), :]
            wi = w32_ref[1, b, pl.ds(k0, 8, stride=5), :]
            yr, yi = ys[b]
            zs.append((yr * wr - yi * wi, yr * wi + yi * wr))
        vs = _fft_list(zs, +1)
        for b in range(N1):
            a_ref[0, pl.ds(r0, 8), pl.ds(b * N2, N2)] = vs[b][0]
            a_ref[1, pl.ds(r0, 8), pl.ds(b * N2, N2)] = vs[b][1]
        return carry

    lax.fori_loop(0, KR // 8, filt, 0)

    cps[6].wait()
    u_ref[:, pl.ds(512, 256)] = jnp.zeros((S, 256), bf)

    def sinv(b, carry):
        c0 = pl.multiple_of(b * N2, N2)
        lhs = li_ref[b]
        for t, (ro, nr) in enumerate(((0, 128), (128, 128), (256, R0))):
            vr = a_ref[0, pl.ds(ro, nr), pl.ds(c0, N2)].astype(bf)
            vi = a_ref[1, pl.ds(ro, nr), pl.ds(c0, N2)].astype(bf)
            pr = lax.dot_general(lhs, vr, nt, preferred_element_type=f32)
            pi = lax.dot_general(lhs, vi, nt, preferred_element_type=f32)
            u_ref[pl.ds(c0, N2), pl.ds(256 * t, nr)] = (
                pr[:N2] - pi[N2:]).astype(bf)
            u_ref[pl.ds(c0, N2), pl.ds(256 * t + 128, nr)] = (
                pi[:N2] + pr[N2:]).astype(bf)
        return carry

    lax.fori_loop(0, N1, sinv, 0)

    cps[7].wait()
    cps[8].wait()
    pq1 = jnp.dot(u_ref[:, pl.ds(0, 256)], gp_ref[0], preferred_element_type=f32)
    pq2 = jnp.dot(u_ref[:, pl.ds(256, 256)], gp_ref[1], preferred_element_type=f32)
    r0_ = jnp.dot(u_ref[:, pl.ds(512, 256)], g0_ref[...], preferred_element_type=f32)
    p1, q1 = pq1[:, :128], pq1[:, 128:]
    p2, q2 = pq2[:, :128], pq2[:, 128:]
    e1 = r0_ + c51 * p1 + c52 * p2
    o1 = s51 * q1 + s52 * q2
    e2 = r0_ + c52 * p1 + c51 * p2
    o2 = s52 * q1 - s51 * q2
    x32_ref[0] = r0_ + p1 + p2
    x32_ref[1] = e1 - o1
    x32_ref[2] = e2 - o2
    x32_ref[3] = e2 + o2
    x32_ref[4] = e1 + o1

    def unperm(m, carry):
        o0 = pl.multiple_of(m * 8, 8)
        yt = jnp.concatenate(
            [jnp.concatenate([x32_ref[c, pl.ds(b * N2 + o0, 8), :]
                              for c in range(5)], axis=1)
             for b in range(N1)], axis=0).astype(bf)
        yo = jnp.dot(pm_ref[1], yt, preferred_element_type=f32)
        oa_ref[pl.ds(pl.multiple_of(m * 128, 128), 128), :] = yo.astype(bf)
        return carry

    lax.fori_loop(0, N1, unperm, 0)
    cp_a = pltpu.make_async_copy(oa_ref, out_hbm.at[:, pl.ds(0, D)],
                                 out_sems.at[NOC])
    cp_a.start()

    cps[9].wait()
    cps[10].wait()
    cps[11].wait()
    bx = bx_ref[...]
    scale = DH ** -0.5 * float(np.log2(np.e))
    wq = wqkv_ref[:, pl.ds(0, D)]
    wk = wqkv_ref[:, pl.ds(D, D)]
    wv = wqkv_ref[:, pl.ds(2 * D, D)]
    tn = (((0,), (1,)), ((), ()))
    qt = lax.dot_general(wq, bx, tn, preferred_element_type=f32)
    vt = lax.dot_general(wv, bx, tn, preferred_element_type=f32)
    kk = jnp.dot(bx, wk, preferred_element_type=f32)

    row_h = (lax.broadcasted_iota(jnp.int32, (D, 128), 0) // DH) % 4
    aug_r = lax.broadcasted_iota(jnp.int32, (128 - GR, 128), 0)
    aug = jnp.where(aug_r == 0, NEG, 0.0).astype(bf)
    for J in range(S // 128):
        blk = qt[:, J * 128:(J + 1) * 128].astype(bf).astype(f32) * scale
        res = blk
        for hl in range(1, 4):
            res = jnp.where(row_h == hl, pltpu.roll(blk, 32 * hl, 1), res)
        for g in range(G):
            rg_ = res[g * GR:(g + 1) * GR]
            for j in range(4):
                qm_ref[j, g, pl.ds(0, GR), pl.ds(J * 128, 128)] = (
                    rg_ * mk_ref[j]).astype(bf)
                qm_ref[j, g, pl.ds(GR, 128 - GR), pl.ds(J * 128, 128)] = aug

    for g in range(G):
        vt_ref[g, pl.ds(0, GR), pl.ds(0, WIN)] = jnp.zeros((GR, WIN), bf)
        vt_ref[g, pl.ds(0, GR), pl.ds(WIN, S)] = vt[g * GR:(g + 1) * GR].astype(bf)

    lane_k = lax.broadcasted_iota(jnp.int32, (WIN, 128), 1)
    pad_rows = jnp.where(lane_k == GR, 1.0, 0.0).astype(bf)
    for g in range(G):
        kg_ref[g, pl.ds(0, WIN), :] = pad_rows
        kg_ref[g, pl.ds(WIN, S), pl.ds(0, GR)] = kk[:, g * GR:(g + 1) * GR].astype(bf)
        kg_ref[g, pl.ds(WIN, S), pl.ds(GR, 128 - GR)] = jnp.zeros((S, 128 - GR), bf)

    r32 = lax.broadcasted_iota(jnp.int32, (QB, 128), 0)
    qi32 = lax.broadcasted_iota(jnp.int32, (QB, 128), 1) % QB
    m_first = r32 > qi32
    m_last = r32 <= qi32
    hrow = lax.broadcasted_iota(jnp.int32, (GR, 128), 0) // DH
    NIT = G * (S // 128)

    def qk(it, sc_ref):
        g = it // (S // 128)
        J = it % (S // 128)
        c0 = pl.multiple_of(J * 128, 128)
        for j in range(4):
            rhs = qm_ref[j, g, :, pl.ds(c0, 128)]
            k0 = pl.multiple_of(J * 128 + 32 * j, 32)
            kwin = kg_ref[g, pl.ds(k0, KW), :]
            st = jnp.dot(kwin, rhs, preferred_element_type=f32)
            sc_ref[j, pl.ds(0, QB), :] = jnp.where(m_first, st[:QB], NEG)
            sc_ref[j, pl.ds(QB, WIN - QB), :] = st[QB:WIN]
            sc_ref[j, pl.ds(WIN, QB), :] = jnp.where(m_last, st[WIN:], NEG)

    def sm_pv(it, sc_ref):
        g = it // (S // 128)
        J = it % (S // 128)
        c0 = pl.multiple_of(J * 128, 128)
        rg = pl.multiple_of(g * GR, 16)
        vwin = vt_ref[g, :, pl.ds(c0, 384)]
        oacc = jnp.zeros((GR, 128), f32)
        for j in range(4):
            st = sc_ref[j]
            m = jnp.max(st, axis=0, keepdims=True)
            p = jnp.exp2(st - m)
            l = jnp.sum(p, axis=0, keepdims=True)
            oj = jnp.dot(vwin[:, 32 * j:32 * j + KW], p.astype(bf),
                         preferred_element_type=f32)
            oj = oj * (1.0 / l)
            oacc = oacc + oj * mk_ref[j]
        res = oacc
        for hl in range(1, 4):
            res = jnp.where(hrow == hl, pltpu.roll(oacc, 128 - 32 * hl, 1), res)
        ot_ref[pl.ds(rg, GR), pl.ds(c0, 128)] = res.astype(bf)

    qk(0, sc0_ref)

    def attn(t, carry):
        it = 2 * t
        qk(it + 1, sc1_ref)
        sm_pv(it, sc0_ref)
        qk(jnp.minimum(it + 2, NIT - 1), sc0_ref)
        sm_pv(it + 1, sc1_ref)
        return carry

    lax.fori_loop(0, NIT // 2, attn, 0)

    cps[12].wait()
    t0 = (((0,), (0,)), ((), ()))
    OC = S // NOC
    cp_b = []
    for c in range(NOC):
        yb = lax.dot_general(ot_ref[:, pl.ds(c * OC, OC)], wo_ref[...], t0,
                             preferred_element_type=f32)
        ob_ref[pl.ds(c * OC, OC), :] = yb.astype(bf)
        cp = pltpu.make_async_copy(
            ob_ref.at[pl.ds(c * OC, OC), :],
            out_hbm.at[pl.ds(c * OC, OC), pl.ds(D, D)], out_sems.at[c])
        cp.start()
        cp_b.append(cp)
    cp_a.wait()
    for cp in cp_b:
        cp.wait()


@jax.jit
def pallas_concat_heads__spectral_gfnet__sliding_block__prompt_kernel(
    A_x: jax.Array,
    A_w_r: jax.Array,
    A_w_i: jax.Array,
    B_x: jax.Array,
    B_wqkv: jax.Array,
    B_wo: jax.Array,
):
    fp, f0, gp, g0, rf, li, mk, pm = _constants()
    f32 = jnp.float32
    bf = jnp.bfloat16
    out = pl.pallas_call(
        _kernel,
        out_shape=jax.ShapeDtypeStruct((S, 2 * D), bf),
        in_specs=[pl.BlockSpec(memory_space=pl.ANY)] * 14,
        out_specs=pl.BlockSpec(memory_space=pl.ANY),
        scratch_shapes=[
            pltpu.VMEM((S, D), bf),
            pltpu.VMEM((DF, S), bf),
            pltpu.VMEM((DF, S), bf),
            pltpu.VMEM((S, D), bf),
            pltpu.VMEM((D, 3 * D), bf),
            pltpu.VMEM((D, D), bf),
            pltpu.VMEM(fp.shape, bf),
            pltpu.VMEM(f0.shape, bf),
            pltpu.VMEM(gp.shape, bf),
            pltpu.VMEM(g0.shape, bf),
            pltpu.VMEM(rf.shape, bf),
            pltpu.VMEM(li.shape, bf),
            pltpu.VMEM(mk.shape, f32),
            pltpu.VMEM(pm.shape, bf),
            pltpu.VMEM((S, D), bf),
            pltpu.VMEM((S, D), bf),
            pltpu.SemaphoreType.DMA((13,)),
            pltpu.SemaphoreType.DMA((NOC + 1,)),
            pltpu.SemaphoreType.DMA((NXC,)),
            pltpu.VMEM((5, S, 128), f32),
            pltpu.VMEM((S, D), f32),
            pltpu.VMEM((2 * KR, S), bf),
            pltpu.VMEM((2, KR, S), f32),
            pltpu.VMEM((2, N1, WR, N2), f32),
            pltpu.VMEM((S, 768), bf),
            pltpu.VMEM((4, G, 128, S), bf),
            pltpu.VMEM((G, VR, SP), bf),
            pltpu.VMEM((G, SP, 128), bf),
            pltpu.VMEM((D, S), bf),
            pltpu.VMEM((4, KW, 128), f32),
            pltpu.VMEM((4, KW, 128), f32),
        ],
        compiler_params=pltpu.CompilerParams(
            vmem_limit_bytes=100 * 1024 * 1024),
    )(A_x.reshape(S, D), A_w_r.T, A_w_i.T, B_x.reshape(S, D), B_wqkv, B_wo,
      fp, f0, gp, g0, rf, li, mk, pm)
    return out.reshape(1, S, 2 * D)
```

```python
import numpy as np
import jax
import jax.numpy as jnp
from jax import lax
import jax.experimental.pallas as pl
import jax.experimental.pallas.tpu as pltpu

S = 2048
D = 640
DF = D // 2 + 1
H = 32
DH = 20
WIN = 256
N1 = 16
N2 = 128
G = 8
GR = 4 * DH
QB = 32
KW = WIN + QB
SP = S + WIN
NEG = -1e9
NXC = 8
R0 = 72
KR = 256 + R0
WR = 5 * R0
NOC = 16


def _constants():
    th = 2.0 * np.pi / D
    rows14 = np.concatenate([1 + 5 * np.arange(64), 4 + 5 * np.arange(64)])
    rows23 = np.concatenate([2 + 5 * np.arange(64), 3 + 5 * np.arange(64)])
    rows0 = 5 * np.arange(R0)
    ok0 = (rows0 <= D // 2).astype(np.float64)
    d2 = np.arange(128)
    sg = np.concatenate([np.ones(64), -np.ones(64)])

    def fwd_pair(rows):
        a = th * ((rows[:, None] * d2[None, :]) % D)
        c, sn = np.cos(a), np.sin(a)
        m = np.zeros((256, 256))
        m[:128, :128] = c
        m[:128, 128:] = sg[:, None] * sn
        m[128:, :128] = -sn
        m[128:, 128:] = sg[:, None] * c
        return m

    def inv_pair(rows):
        a = th * ((rows[:, None] * d2[None, :]) % D)
        c, sn = 2.0 * np.cos(a), 2.0 * np.sin(a)
        m = np.zeros((256, 256))
        m[:128, :128] = c
        m[128:, :128] = -sn
        m[:128, 128:] = sg[:, None] * sn
        m[128:, 128:] = sg[:, None] * c
        return m / (S * D)

    fp = np.stack([fwd_pair(rows14), fwd_pair(rows23)])
    gp = np.stack([inv_pair(rows14), inv_pair(rows23)])
    a0 = th * ((rows0[:, None] * d2[None, :]) % D)
    f0 = np.concatenate([np.cos(a0), -np.sin(a0)]) * np.tile(ok0, 2)[:, None]
    c0 = 2.0 * ok0.copy()
    c0[0] = 1.0
    c0[D // 2 // 5] = 1.0
    s0 = c0.copy()
    s0[0] = 0.0
    s0[D // 2 // 5] = 0.0
    g0 = np.zeros((256, 128))
    g0[:R0] = c0[:, None] * np.cos(a0)
    g0[128:128 + R0] = -s0[:, None] * np.sin(a0)
    g0 = g0 / (S * D)
    s1 = np.arange(N2)[:, None]
    k1 = np.arange(N2)[None, :]
    rf = np.zeros((N1, N2, 2 * N2))
    li = np.zeros((N1, 2 * N2, N2))
    for b in range(N1):
        a = 2.0 * np.pi * (((N1 * s1 + b) * k1) % S) / S
        rf[b, :, :N2] = np.cos(a)
        rf[b, :, N2:] = np.sin(a)
        li[b, :N2] = np.cos(a)
        li[b, N2:] = np.sin(a)
    pm = np.zeros((2, 128, 128))
    for b in range(N1):
        for l in range(8):
            pm[0, b * 8 + l, l * 16 + b] = 1.0
    pm[1] = pm[0].T
    hrow = (np.arange(GR) // DH)[:, None]
    slot = (np.arange(128) // QB)[None, :]
    mk = np.stack([(slot == (hrow + j) % 4) for j in range(4)]).astype(np.float32)
    bf = jnp.bfloat16
    return (jnp.asarray(fp, bf), jnp.asarray(f0, bf), jnp.asarray(gp, bf),
            jnp.asarray(g0, bf), jnp.asarray(rf, bf), jnp.asarray(li, bf),
            jnp.asarray(mk), jnp.asarray(pm, bf))


def _cmul_const(re, im, k, n, sign):
    k = k % n
    if k == 0:
        return re, im
    if 4 * k == n:
        return (-im, re) if sign > 0 else (im, -re)
    if 2 * k == n:
        return -re, -im
    if 4 * k == 3 * n:
        return (im, -re) if sign > 0 else (-im, re)
    c = float(np.cos(2 * np.pi * k / n))
    s = float(np.sin(2 * np.pi * k / n)) * sign
    if abs(abs(c) - abs(s)) < 1e-12:
        if s * c > 0:
            return (re - im) * c, (re + im) * c
        return (re + im) * c, (im - re) * c
    return re * c - im * s, re * s + im * c


def _fft_list(xs, sign):
    n = len(xs)
    if n == 1:
        return xs
    ev = _fft_list(xs[0::2], sign)
    od = _fft_list(xs[1::2], sign)
    out = [None] * n
    for k in range(n // 2):
        tr, ti = _cmul_const(od[k][0], od[k][1], k, n, sign)
        out[k] = (ev[k][0] + tr, ev[k][1] + ti)
        out[k + n // 2] = (ev[k][0] - tr, ev[k][1] - ti)
    return out


def _kernel(ax_hbm, wr_hbm, wi_hbm, bx_hbm, wqkv_hbm, wo_hbm,
            fp_hbm, f0_hbm, gp_hbm, g0_hbm, rf_hbm, li_hbm, mk_hbm, pm_hbm,
            out_hbm,
            ax_ref, wr_ref, wi_ref, bx_ref, wqkv_ref, wo_ref,
            fp_ref, f0_ref, gp_ref, g0_ref, rf_ref, li_ref, mk_ref, pm_ref,
            oa_ref, ob_ref, in_sems, out_sems, x_sems,
            x32_ref, tt_ref, xt_ref, a_ref, w32_ref, u_ref,
            qm_ref, vt_ref, kg_ref, ot_ref, sc0_ref, sc1_ref):
    f32 = jnp.float32
    bf = jnp.bfloat16

    XC = S // NXC

    def x_copy(c):
        return pltpu.make_async_copy(ax_hbm.at[pl.ds(c * XC, XC), :],
                                     ax_ref.at[pl.ds(c * XC, XC), :],
                                     x_sems.at[c])

    srcs = (pm_hbm, fp_hbm, f0_hbm, rf_hbm, wr_hbm, wi_hbm, li_hbm, gp_hbm,
            g0_hbm, bx_hbm, wqkv_hbm, mk_hbm, wo_hbm)
    dsts = (pm_ref, fp_ref, f0_ref, rf_ref, wr_ref, wi_ref, li_ref, gp_ref,
            g0_ref, bx_ref, wqkv_ref, mk_ref, wo_ref)
    cps = [pltpu.make_async_copy(s_, d_, in_sems.at[i])
           for i, (s_, d_) in enumerate(zip(srcs, dsts))]
    cps[0].start()
    for c in range(NXC):
        x_copy(c).start()
    for c_ in cps[1:4]:
        c_.start()

    c51 = float(np.cos(2 * np.pi / 5))
    c52 = float(np.cos(4 * np.pi / 5))
    s51 = float(np.sin(2 * np.pi / 5))
    s52 = float(np.sin(4 * np.pi / 5))
    nt = (((1,), (1,)), ((), ()))

    cps[0].wait()

    def rad5(m, carry):
        r0 = pl.multiple_of(m * 128, 128)
        xp = jnp.dot(pm_ref[0], ax_ref[pl.ds(r0, 128), :],
                     preferred_element_type=f32)
        xs = [xp[:, c * 128:(c + 1) * 128] for c in range(5)]
        a1 = xs[1] + xs[4]
        b1 = xs[1] - xs[4]
        a2 = xs[2] + xs[3]
        b2 = xs[2] - xs[3]
        ts = jnp.concatenate(
            (xs[0] + a1 + a2,
             xs[0] + c51 * a1 + c52 * a2,
             -(s51 * b1 + s52 * b2),
             xs[0] + c52 * a1 + c51 * a2,
             s51 * b2 - s52 * b1), axis=1)
        o0 = pl.multiple_of(m * 8, 8)
        for b in range(N1):
            tt_ref[pl.ds(b * N2 + o0, 8), :] = ts[b * 8:(b + 1) * 8]
        return carry

    for c in range(NXC):
        x_copy(c).wait()
        if c == NXC - 1:
            for c_ in cps[4:9]:
                c_.start()
        lax.fori_loop(c * (N1 // NXC), (c + 1) * (N1 // NXC), rad5, 0, unroll=True)
    for c_ in cps[9:]:
        c_.start()

    cps[1].wait()
    cps[2].wait()
    for p_ in range(2):
        xp = lax.dot_general(
            fp_ref[p_], tt_ref[:, pl.ds(128 + 256 * p_, 256)].astype(bf),
            nt, preferred_element_type=f32)
        xt_ref[pl.ds(128 * p_, 128), :] = xp[:128].astype(bf)
        xt_ref[pl.ds(KR + 128 * p_, 128), :] = xp[128:].astype(bf)
    x0 = lax.dot_general(f0_ref[...], tt_ref[:, pl.ds(0, 128)].astype(bf), nt,
                         preferred_element_type=f32)
    xt_ref[pl.ds(256, R0), :] = x0[:R0].astype(bf)
    xt_ref[pl.ds(KR + 256, R0), :] = x0[R0:].astype(bf)

    cps[3].wait()

    def sfwd(b, carry):
        c0 = pl.multiple_of(b * N2, N2)
        pq = jnp.dot(xt_ref[:, pl.ds(c0, N2)], rf_ref[b],
                     preferred_element_type=f32)
        a_ref[0, :, pl.ds(c0, N2)] = pq[:KR, :N2] + pq[KR:, N2:]
        a_ref[1, :, pl.ds(c0, N2)] = pq[KR:, :N2] - pq[:KR, N2:]
        return carry

    lax.fori_loop(0, N1, sfwd, 0, unroll=True)

    cps[4].wait()
    cps[5].wait()
    for p_, w_ref in enumerate((wr_ref, wi_ref)):
        for b in range(N1):
            w32_ref[p_, b, pl.ds(0, DF), :] = (
                w_ref[:, pl.ds(b * N2, N2)].astype(f32))
            w32_ref[p_, b, pl.ds(DF, WR - DF), :] = jnp.zeros((WR - DF, N2), f32)

    def filt(i, carry):
        r0 = pl.multiple_of(i * 8, 8)
        grp = i // 8
        k1 = jnp.where(grp == 0, 1, jnp.where(grp == 1, 4, jnp.where(
            grp == 2, 2, jnp.where(grp == 3, 3, 0))))
        jj = jnp.where(grp >= 4, r0 - 256, r0 - grp * 64)
        k0 = k1 + 5 * jj
        xs = [(a_ref[0, pl.ds(r0, 8), pl.ds(b * N2, N2)],
               a_ref[1, pl.ds(r0, 8), pl.ds(b * N2, N2)]) for b in range(N1)]
        ys = _fft_list(xs, -1)
        zs = []
        for b in range(N1):
            wr = w32_ref[0, b, pl.ds(k0, 8, stride=5), :]
            wi = w32_ref[1, b, pl.ds(k0, 8, stride=5), :]
            yr, yi = ys[b]
            zs.append((yr * wr - yi * wi, yr * wi + yi * wr))
        vs = _fft_list(zs, +1)
        for b in range(N1):
            a_ref[0, pl.ds(r0, 8), pl.ds(b * N2, N2)] = vs[b][0]
            a_ref[1, pl.ds(r0, 8), pl.ds(b * N2, N2)] = vs[b][1]
        return carry

    lax.fori_loop(0, KR // 8, filt, 0)

    cps[6].wait()
    u_ref[:, pl.ds(512, 256)] = jnp.zeros((S, 256), bf)

    def sinv(b, carry):
        c0 = pl.multiple_of(b * N2, N2)
        lhs = li_ref[b]
        for t, (ro, nr) in enumerate(((0, 128), (128, 128), (256, R0))):
            vr = a_ref[0, pl.ds(ro, nr), pl.ds(c0, N2)].astype(bf)
            vi = a_ref[1, pl.ds(ro, nr), pl.ds(c0, N2)].astype(bf)
            pr = lax.dot_general(lhs, vr, nt, preferred_element_type=f32)
            pi = lax.dot_general(lhs, vi, nt, preferred_element_type=f32)
            u_ref[pl.ds(c0, N2), pl.ds(256 * t, nr)] = (
                pr[:N2] - pi[N2:]).astype(bf)
            u_ref[pl.ds(c0, N2), pl.ds(256 * t + 128, nr)] = (
                pi[:N2] + pr[N2:]).astype(bf)
        return carry

    lax.fori_loop(0, N1, sinv, 0, unroll=True)

    cps[7].wait()
    cps[8].wait()
    pq1 = jnp.dot(u_ref[:, pl.ds(0, 256)], gp_ref[0], preferred_element_type=f32)
    pq2 = jnp.dot(u_ref[:, pl.ds(256, 256)], gp_ref[1], preferred_element_type=f32)
    r0_ = jnp.dot(u_ref[:, pl.ds(512, 256)], g0_ref[...], preferred_element_type=f32)
    p1, q1 = pq1[:, :128], pq1[:, 128:]
    p2, q2 = pq2[:, :128], pq2[:, 128:]
    e1 = r0_ + c51 * p1 + c52 * p2
    o1 = s51 * q1 + s52 * q2
    e2 = r0_ + c52 * p1 + c51 * p2
    o2 = s52 * q1 - s51 * q2
    x32_ref[0] = r0_ + p1 + p2
    x32_ref[1] = e1 - o1
    x32_ref[2] = e2 - o2
    x32_ref[3] = e2 + o2
    x32_ref[4] = e1 + o1

    def unperm(m, carry):
        o0 = pl.multiple_of(m * 8, 8)
        yt = jnp.concatenate(
            [jnp.concatenate([x32_ref[c, pl.ds(b * N2 + o0, 8), :]
                              for c in range(5)], axis=1)
             for b in range(N1)], axis=0).astype(bf)
        yo = jnp.dot(pm_ref[1], yt, preferred_element_type=f32)
        oa_ref[pl.ds(pl.multiple_of(m * 128, 128), 128), :] = yo.astype(bf)
        return carry

    lax.fori_loop(0, N1, unperm, 0, unroll=True)
    cp_a = pltpu.make_async_copy(oa_ref, out_hbm.at[:, pl.ds(0, D)],
                                 out_sems.at[NOC])
    cp_a.start()

    cps[9].wait()
    cps[10].wait()
    cps[11].wait()
    bx = bx_ref[...]
    scale = DH ** -0.5 * float(np.log2(np.e))
    wq = wqkv_ref[:, pl.ds(0, D)]
    wk = wqkv_ref[:, pl.ds(D, D)]
    wv = wqkv_ref[:, pl.ds(2 * D, D)]
    tn = (((0,), (1,)), ((), ()))
    qt = lax.dot_general(wq, bx, tn, preferred_element_type=f32)
    vt = lax.dot_general(wv, bx, tn, preferred_element_type=f32)
    kk = jnp.dot(bx, wk, preferred_element_type=f32)

    row_h = (lax.broadcasted_iota(jnp.int32, (D, 128), 0) // DH) % 4
    for J in range(S // 128):
        blk = qt[:, J * 128:(J + 1) * 128].astype(bf).astype(f32) * scale
        res = blk
        for hl in range(1, 4):
            res = jnp.where(row_h == hl, pltpu.roll(blk, 32 * hl, 1), res)
        for g in range(G):
            rg_ = res[g * GR:(g + 1) * GR]
            for j in range(4):
                qm_ref[j, g, :, pl.ds(J * 128, 128)] = (
                    rg_ * mk_ref[j]).astype(bf)

    for g in range(G):
        vt_ref[g, pl.ds(0, GR), pl.ds(0, WIN)] = jnp.zeros((GR, WIN), bf)
        vt_ref[g, pl.ds(0, GR), pl.ds(WIN, S)] = vt[g * GR:(g + 1) * GR].astype(bf)

    for g in range(G):
        kg_ref[g] = kk[:, g * GR:(g + 1) * GR].astype(bf)

    r32 = lax.broadcasted_iota(jnp.int32, (QB, 128), 0)
    qi32 = lax.broadcasted_iota(jnp.int32, (QB, 128), 1) % QB
    m_first = r32 > qi32
    m_last = r32 <= qi32
    hrow = lax.broadcasted_iota(jnp.int32, (GR, 128), 0) // DH

    def qk(g, J, sc_ref):
        c0 = J * 128
        for j in range(4):
            k0 = J * 128 + 32 * j
            lo = max(0, WIN - k0)
            rhs = qm_ref[j, g, :, pl.ds(c0, 128)]
            kwin = kg_ref[g, pl.ds(k0 + lo - WIN, KW - lo), :]
            st = jnp.dot(kwin, rhs, preferred_element_type=f32)
            if lo == 0:
                sc_ref[j, pl.ds(0, QB), :] = jnp.where(m_first, st[:QB], NEG)
                sc_ref[j, pl.ds(QB, WIN - QB), :] = st[QB:WIN]
            elif lo < WIN:
                sc_ref[j, pl.ds(lo, WIN - lo), :] = st[:WIN - lo]
            sc_ref[j, pl.ds(WIN, QB), :] = jnp.where(
                m_last, st[WIN - lo:], NEG)

    def sm_pv(g, J, sc_ref):
        c0 = J * 128
        rg = pl.multiple_of(g * GR, 16)
        vwin = vt_ref[g, :, pl.ds(c0, 384)]
        oacc = jnp.zeros((GR, 128), f32)
        for j in range(4):
            lo = max(0, WIN - (J * 128 + 32 * j))
            st = sc_ref[j, pl.ds(lo, KW - lo), :]
            m = jnp.max(st, axis=0, keepdims=True)
            p = jnp.exp2(st - m)
            l = jnp.sum(p, axis=0, keepdims=True)
            oj = jnp.dot(vwin[:, 32 * j + lo:32 * j + KW], p.astype(bf),
                         preferred_element_type=f32)
            oj = oj * (1.0 / l)
            oacc = oacc + oj * mk_ref[j]
        res = oacc
        for hl in range(1, 4):
            res = jnp.where(hrow == hl, pltpu.roll(oacc, 128 - 32 * hl, 1), res)
        ot_ref[pl.ds(rg, GR), pl.ds(c0, 128)] = res.astype(bf)

    qk(0, 0, sc0_ref)
    NJ = S // 128

    def attn(g, carry):
        bufs = (sc0_ref, sc1_ref)
        for J in range(NJ):
            if J + 1 < NJ:
                qk(g, J + 1, bufs[(J + 1) % 2])
            else:
                qk(jnp.minimum(g + 1, G - 1), 0, bufs[0])
            sm_pv(g, J, bufs[J % 2])
        return carry

    lax.fori_loop(0, G, attn, 0)

    cps[12].wait()
    t0 = (((0,), (0,)), ((), ()))
    OC = S // NOC
    cp_b = []
    for c in range(NOC):
        yb = lax.dot_general(ot_ref[:, pl.ds(c * OC, OC)], wo_ref[...], t0,
                             preferred_element_type=f32)
        ob_ref[pl.ds(c * OC, OC), :] = yb.astype(bf)
        cp = pltpu.make_async_copy(
            ob_ref.at[pl.ds(c * OC, OC), :],
            out_hbm.at[pl.ds(c * OC, OC), pl.ds(D, D)], out_sems.at[c])
        cp.start()
        cp_b.append(cp)
    cp_a.wait()
    for cp in cp_b:
        cp.wait()


@jax.jit
def pallas_concat_heads__spectral_gfnet__sliding_block__prompt_kernel(
    A_x: jax.Array,
    A_w_r: jax.Array,
    A_w_i: jax.Array,
    B_x: jax.Array,
    B_wqkv: jax.Array,
    B_wo: jax.Array,
):
    fp, f0, gp, g0, rf, li, mk, pm = _constants()
    f32 = jnp.float32
    bf = jnp.bfloat16
    out = pl.pallas_call(
        _kernel,
        out_shape=jax.ShapeDtypeStruct((S, 2 * D), bf),
        in_specs=[pl.BlockSpec(memory_space=pl.ANY)] * 14,
        out_specs=pl.BlockSpec(memory_space=pl.ANY),
        scratch_shapes=[
            pltpu.VMEM((S, D), bf),
            pltpu.VMEM((DF, S), bf),
            pltpu.VMEM((DF, S), bf),
            pltpu.VMEM((S, D), bf),
            pltpu.VMEM((D, 3 * D), bf),
            pltpu.VMEM((D, D), bf),
            pltpu.VMEM(fp.shape, bf),
            pltpu.VMEM(f0.shape, bf),
            pltpu.VMEM(gp.shape, bf),
            pltpu.VMEM(g0.shape, bf),
            pltpu.VMEM(rf.shape, bf),
            pltpu.VMEM(li.shape, bf),
            pltpu.VMEM(mk.shape, f32),
            pltpu.VMEM(pm.shape, bf),
            pltpu.VMEM((S, D), bf),
            pltpu.VMEM((S, D), bf),
            pltpu.SemaphoreType.DMA((13,)),
            pltpu.SemaphoreType.DMA((NOC + 1,)),
            pltpu.SemaphoreType.DMA((NXC,)),
            pltpu.VMEM((5, S, 128), f32),
            pltpu.VMEM((S, D), f32),
            pltpu.VMEM((2 * KR, S), bf),
            pltpu.VMEM((2, KR, S), f32),
            pltpu.VMEM((2, N1, WR, N2), f32),
            pltpu.VMEM((S, 768), bf),
            pltpu.VMEM((4, G, GR, S), bf),
            pltpu.VMEM((G, GR, SP), bf),
            pltpu.VMEM((G, S, GR), bf),
            pltpu.VMEM((D, S), bf),
            pltpu.VMEM((4, KW, 128), f32),
            pltpu.VMEM((4, KW, 128), f32),
        ],
        compiler_params=pltpu.CompilerParams(
            vmem_limit_bytes=100 * 1024 * 1024),
    )(A_x.reshape(S, D), A_w_r.T, A_w_i.T, B_x.reshape(S, D), B_wqkv, B_wo,
      fp, f0, gp, g0, rf, li, mk, pm)
    return out.reshape(1, S, 2 * D)
```
